```python
import jax
import jax.numpy as jnp

def _softmax(x, axis=-1):
    return jax.nn.softmax(x, axis=axis)
def _gelu(x):
    return jax.nn.gelu(x, approximate=True)
def _silu(x):
    return jax.nn.silu(x)
def _sigmoid(x):
    return jax.nn.sigmoid(x)
def _layernorm(x, axis=-1, eps=1e-5):
    m = jnp.mean(x, axis=axis, keepdims=True)
    v = jnp.var(x, axis=axis, keepdims=True)
    return (x - m) / jnp.sqrt(v + eps)
def _scatter_add(tgt, idx, src, axis=0):
    return tgt.at[idx].add(src)
def _segment_sum(src, seg, n):
    return jax.ops.segment_sum(src, seg, n)
class _Rng:
    def __init__(self, key):
        self._k = key
    def _next(self):
        self._k, sub = jax.random.split(self._k)
        return sub
    def normal(self, shape):
        return jax.random.normal(self._next(), shape, dtype=jnp.bfloat16)
    def randint(self, lo, hi, shape):
        return jax.random.randint(self._next(), shape, lo, hi, dtype=jnp.int32)
    def uniform(self, shape, lo=0.0, hi=1.0):
        return jax.random.uniform(self._next(), shape, jnp.bfloat16, lo, hi)
    def permutation(self, n):
        return jax.random.permutation(self._next(), n)


kernel_name = 'concat_heads__mha_block_cached__gqa_block_cached__near_ridge'

def _fwd_setup_inputs():
    _rng = _Rng(jax.random.key(int.from_bytes(__import__("os").urandom(4), "little")))
    _w = (lambda a: (lambda t: t.astype(jnp.bfloat16) if jnp.issubdtype(t.dtype, jnp.floating) else t)(jnp.asarray(a)))
    def _A_setup():
        B, Sq, D = 8, 224, 448
        H, Sk, Dh = 16, 512, 256
        return {
            "x": _w((lambda *s: _rng.normal(s) * 0.05)(B, Sq, D)),
            "k_cache": _w((lambda *s: _rng.normal(s) * 0.05)(B, H, Sk, Dh)),
            "v_cache": _w((lambda *s: _rng.normal(s) * 0.05)(B, H, Sk, Dh)),
            "wq": _w((lambda *s: _rng.normal(s) * 0.05)(D, H * Dh) * (D ** -0.5)),
            "wo": _w((lambda *s: _rng.normal(s) * 0.05)(H * Dh, D) * ((H * Dh) ** -0.5)),
        }
    _A_in = _A_setup()

    def _B_setup():
        B, Sq, D = 8, 224, 448
        Hq, Hkv, Sk, Dh = 16, 16, 512, 256
        assert Hq % Hkv == 0, (Hq, Hkv)
        return {
            "x": _w((lambda *s: _rng.normal(s) * 0.05)(B, Sq, D)),
            "k_cache": _w((lambda *s: _rng.normal(s) * 0.05)(B, Hkv, Sk, Dh)),
            "v_cache": _w((lambda *s: _rng.normal(s) * 0.05)(B, Hkv, Sk, Dh)),
            "wq": _w((lambda *s: _rng.normal(s) * 0.05)(D, Hq * Dh) * (D ** -0.5)),
            "wo": _w((lambda *s: _rng.normal(s) * 0.05)(Hq * Dh, D) * ((Hq * Dh) ** -0.5)),
        }
    _B_in = _B_setup()

    return {
        "A_x": _A_in["x"],
        "A_k_cache": _A_in["k_cache"],
        "A_v_cache": _A_in["v_cache"],
        "A_wq": _A_in["wq"],
        "A_wo": _A_in["wo"],
        "B_x": _B_in["x"],
        "B_k_cache": _B_in["k_cache"],
        "B_v_cache": _B_in["v_cache"],
        "B_wq": _B_in["wq"],
        "B_wo": _B_in["wo"],
    }

def _fwd_reference(A_x, A_k_cache, A_v_cache, A_wq, A_wo, B_x, B_k_cache, B_v_cache, B_wq, B_wo):
    def _A_ref(x, k_cache, v_cache, wq, wo):
        B, Sq, D = x.shape
        H, Dh = 16, 256
        q = (lambda x, *d: x.transpose(*d))((x @ wq).reshape(B, Sq, H, Dh), 0, 2, 1, 3)
        scores = jnp.einsum("bhqd,bhkd->bhqk", q, k_cache) * (Dh ** -0.5)
        p = _softmax(scores, axis=-1)
        o = jnp.einsum("bhqk,bhkd->bhqd", p, v_cache)
        return (lambda x, *d: x.transpose(*d))(o, 0, 2, 1, 3).reshape(B, Sq, H * Dh) @ wo

    def _B_ref(x, k_cache, v_cache, wq, wo):
        B, Sq, D = x.shape
        Hq, Dh = 16, 256
        Hkv = k_cache.shape[1]
        rep = Hq // Hkv
        q = (lambda x, *d: x.transpose(*d))((x @ wq).reshape(B, Sq, Hq, Dh), 0, 2, 1, 3)
        k = jnp.repeat(k_cache, rep, axis=1)
        v = jnp.repeat(v_cache, rep, axis=1)
        scores = jnp.einsum("bhqd,bhkd->bhqk", q, k) * (Dh ** -0.5)
        p = _softmax(scores, axis=-1)
        o = jnp.einsum("bhqk,bhkd->bhqd", p, v)
        return (lambda x, *d: x.transpose(*d))(o, 0, 2, 1, 3).reshape(B, Sq, Hq * Dh) @ wo

    a = _A_ref(A_x, A_k_cache, A_v_cache, A_wq, A_wo)
    b = _B_ref(B_x, B_k_cache, B_v_cache, B_wq, B_wo)
    return jnp.concatenate([a, b], axis=-1)


def setup_inputs():
    _inp = _fwd_setup_inputs()
    _gk = jax.random.fold_in(jax.random.key(int.from_bytes(__import__("os").urandom(4), "little")), 2**31 - 1)
    _shapes = [[8, 224, 896]]
    _dtypes = ['bfloat16']
    _gks = jax.random.split(_gk, len(_shapes))
    _gs = [jax.random.normal(k, s, dtype=jnp.dtype(d)) * 0.05 for k, s, d in zip(_gks, _shapes, _dtypes)]
    _inp["grad_out"] = _gs[0]
    return _inp

def reference(A_x, A_k_cache, A_v_cache, A_wq, A_wo, B_x, B_k_cache, B_v_cache, B_wq, B_wo, grad_out):
    _const = dict()
    def _f(*_d):
        return _fwd_reference(**{'A_x': _d[0], 'A_k_cache': _d[1], 'A_v_cache': _d[2], 'A_wq': _d[3], 'A_wo': _d[4], 'B_x': _d[5], 'B_k_cache': _d[6], 'B_v_cache': _d[7], 'B_wq': _d[8], 'B_wo': _d[9], **_const})
    _out, _vjp = jax.vjp(_f, A_x, A_k_cache, A_v_cache, A_wq, A_wo, B_x, B_k_cache, B_v_cache, B_wq, B_wo)
    _grads = _vjp(grad_out)
    _out0 = jnp.asarray(_out)
    return (_out0, *[jnp.asarray(_g) for _g in _grads])
```

```python
import functools
import jax
import jax.numpy as jnp
from jax import lax
import jax.experimental.pallas as pl
import jax.experimental.pallas.tpu as pltpu

B, SQ, D, H, SK, DH = 8, 224, 448, 16, 512, 256
R = B * SQ
SCALE = DH ** -0.5
BF, F32 = jnp.bfloat16, jnp.float32
NN = (((1,), (0,)), ((), ()))
NT = (((1,), (1,)), ((), ()))
TN = (((0,), (0,)), ((), ()))


def _dot(a, b, dn):
    return lax.dot_general(a, b, dn, preferred_element_type=F32)


def make_kernel(mode="plain", unroll=8):
    def kernel(xa, ka, va, wqa, woa, xb, kb, vb, wqb, wob, g_hbm,
               out_hbm, dxa, dka, dva, dwqa, dwoa, dxb, dkb, dvb, dwqb, dwob,
               x_s, g_s, xt_s, gt_s, graw_s,
               k_s, v_s, wq_s, wo_s, dk_s, dv_s, dwq_s, dwo_s,
               q_s, do_s, o_s, dq_s, outT_acc, dxT_acc, out_s, dx_s,
               isem, osem, msem):
        def in_copies(branch, h, slot):
            kh, vh, wqh, woh = (ka, va, wqa, woa) if branch == 0 else (kb, vb, wqb, wob)
            col = pl.ds(pl.multiple_of(h * DH, DH), DH)
            return [
                pltpu.make_async_copy(wqh.at[:, col], wq_s.at[slot], isem.at[0, slot]),
                pltpu.make_async_copy(woh.at[:, col], wo_s.at[slot], isem.at[1, slot]),
                pltpu.make_async_copy(kh.at[:, h], k_s.at[slot], isem.at[2, slot]),
                pltpu.make_async_copy(vh.at[:, h], v_s.at[slot], isem.at[3, slot]),
            ]

        def kv_out_copies(branch, h, slot):
            dkh, dvh = (dka, dva) if branch == 0 else (dkb, dvb)
            return [
                pltpu.make_async_copy(dk_s.at[slot], dkh.at[:, h], osem.at[0, slot]),
                pltpu.make_async_copy(dv_s.at[slot], dvh.at[:, h], osem.at[1, slot]),
            ]

        def w_out_copies(branch, h, slot):
            dwqh, dwoh = (dwqa, dwoa) if branch == 0 else (dwqb, dwob)
            col = pl.ds(pl.multiple_of(h * DH, DH), DH)
            return [
                pltpu.make_async_copy(dwq_s.at[slot], dwqh.at[:, col], osem.at[2, slot]),
                pltpu.make_async_copy(dwo_s.at[slot], dwoh.at[:, col], osem.at[3, slot]),
            ]

        def for_step(t, fn):
            @pl.when(t < H)
            def _():
                fn(0, t)

            @pl.when(t >= H)
            def _():
                fn(1, t - H)

        def start_all(cs):
            for c in cs:
                c.start()

        def wait_all(cs):
            for c in cs:
                c.wait()

        xa_cp = pltpu.make_async_copy(xa, x_s.at[0], msem.at[0])
        g_cp = pltpu.make_async_copy(g_hbm, graw_s, msem.at[1])
        xb_cp = pltpu.make_async_copy(xb, x_s.at[1], msem.at[2])
        xa_cp.start()
        c0 = in_copies(0, 0, 0)
        c0[0].start()
        g_cp.start()
        start_all(c0[1:])
        xb_cp.start()
        xa_cp.wait()
        xt_s[0] = x_s[0].T
        g_cp.wait()
        gt = graw_s[...].T
        gt_s[0] = gt[:D]
        gt_s[1] = gt[D:]
        g_s[0] = graw_s[:, :D]
        g_s[1] = graw_s[:, D:]
        xb_cp.wait()
        xt_s[1] = x_s[1].T

        def attn(b, slot):
            rows = pl.ds(pl.multiple_of(b * SQ, SQ), SQ) if not isinstance(b, int) else slice(b * SQ, (b + 1) * SQ)
            q = q_s[rows, :]
            do = do_s[rows, :]
            k = k_s[slot, b]
            v = v_s[slot, b]
            s = _dot(q, k, NT)
            dp = _dot(do, v, NT)
            m = jnp.max(s, axis=1, keepdims=True)
            e = jnp.exp(s - m)
            l = jnp.sum(e, axis=1, keepdims=True)
            p = e * (1.0 / l)
            delta = jnp.sum(p * dp, axis=1, keepdims=True)
            ds = (p * (dp - delta)).astype(BF)
            pb = p.astype(BF)
            o_s[rows, :] = _dot(pb, v, NN).astype(BF)
            dv_s[slot, b] = _dot(pb, do, TN).astype(BF)
            dq_s[rows, :] = (_dot(ds, k, NN) * SCALE).astype(BF)
            dk_s[slot, b] = _dot(ds, q, TN).astype(BF)

        def step(t, carry):
            slot = t % 2
            br = t // H

            @pl.when(t + 1 < 2 * H)
            def _():
                for_step(t + 1, lambda bb, hh: start_all(in_copies(bb, hh, 1 - slot)))

            wait_all(in_copies(0, 0, slot))

            @pl.when(t >= 2)
            def _():
                wait_all(kv_out_copies(0, 0, slot))
                wait_all(w_out_copies(0, 0, slot))

            @pl.when(t % H == 0)
            def _():
                outT_acc[...] = jnp.zeros_like(outT_acc)
                dxT_acc[...] = jnp.zeros_like(dxT_acc)

            q_s[...] = (_dot(x_s[br], wq_s[slot], NN) * SCALE).astype(BF)
            do_s[...] = _dot(g_s[br], wo_s[slot], NN).astype(BF)
            if unroll == B:
                for b in range(B):
                    attn(b, slot)
            else:
                def body(i, c):
                    for u in range(unroll):
                        attn(i * unroll + u, slot)
                    return c
                lax.fori_loop(0, B // unroll, body, 0)
            for_step(t, lambda bb, hh: start_all(kv_out_copies(bb, hh, slot)))
            outT_acc[...] += _dot(wo_s[slot], o_s[...], NT)
            dxT_acc[...] += _dot(wq_s[slot], dq_s[...], NT)
            dwq_s[slot] = _dot(xt_s[br], dq_s[...], NN).astype(BF)
            dwo_s[slot] = _dot(gt_s[br], o_s[...], NN).astype(BF)
            for_step(t, lambda bb, hh: start_all(w_out_copies(bb, hh, slot)))

            @pl.when(t == H - 1)
            def _():
                out_s[:, :D] = outT_acc[...].astype(BF).T
                dx_s[0] = dxT_acc[...].astype(BF).T
                pltpu.make_async_copy(dx_s.at[0], dxa, msem.at[0]).start()
            return carry

        lax.fori_loop(0, 2 * H, step, 0)
        out_s[:, D:] = outT_acc[...].astype(BF).T
        out_cp = pltpu.make_async_copy(out_s, out_hbm, msem.at[1])
        out_cp.start()
        dx_s[1] = dxT_acc[...].astype(BF).T
        dxb_cp = pltpu.make_async_copy(dx_s.at[1], dxb, msem.at[2])
        dxb_cp.start()
        for sl in range(2):
            wait_all(kv_out_copies(0, 0, sl))
            wait_all(w_out_copies(0, 0, sl))
        pltpu.make_async_copy(dx_s.at[0], dxa, msem.at[0]).wait()
        out_cp.wait()
        dxb_cp.wait()

    return kernel


def build(**kw):
    @jax.jit
    def fn(A_x, A_k_cache, A_v_cache, A_wq, A_wo, B_x, B_k_cache, B_v_cache, B_wq, B_wo, grad_out):
        sds = jax.ShapeDtypeStruct
        br_out = [sds((R, D), BF), sds((B, H, SK, DH), BF), sds((B, H, SK, DH), BF),
                  sds((D, H * DH), BF), sds((D, H * DH), BF)]
        any_spec = pl.BlockSpec(memory_space=pl.ANY)
        V = pltpu.VMEM
        scratch = [
            V((2, R, D), BF), V((2, R, D), BF), V((2, D, R), BF), V((2, D, R), BF), V((R, 2 * D), BF),
            V((2, B, SK, DH), BF), V((2, B, SK, DH), BF), V((2, D, DH), BF), V((2, D, DH), BF),
            V((2, B, SK, DH), BF), V((2, B, SK, DH), BF), V((2, D, DH), BF), V((2, D, DH), BF),
            V((R, DH), BF), V((R, DH), BF), V((R, DH), BF), V((R, DH), BF),
            V((D, R), F32), V((D, R), F32), V((R, 2 * D), BF), V((2, R, D), BF),
            pltpu.SemaphoreType.DMA((4, 2)), pltpu.SemaphoreType.DMA((4, 2)), pltpu.SemaphoreType.DMA((3,)),
        ]
        res = pl.pallas_call(
            make_kernel(**kw),
            out_shape=[sds((R, 2 * D), BF)] + br_out + br_out,
            in_specs=[any_spec] * 11,
            out_specs=[any_spec] * 11,
            scratch_shapes=scratch,
            compiler_params=pltpu.CompilerParams(vmem_limit_bytes=110 * 2 ** 20),
        )(A_x.reshape(R, D), A_k_cache, A_v_cache, A_wq, A_wo.T,
          B_x.reshape(R, D), B_k_cache, B_v_cache, B_wq, B_wo.T, grad_out.reshape(R, 2 * D))
        out, dxa, dka, dva, dwqa, dwoa, dxb, dkb, dvb, dwqb, dwob = res
        return (out.reshape(B, SQ, 2 * D), dxa.reshape(B, SQ, D), dka, dva, dwqa, dwoa.T,
                dxb.reshape(B, SQ, D), dkb, dvb, dwqb, dwob.T)
    return fn


pallas_concat_heads__mha_block_cached__gqa_block_cached__near_ridge_kernel = build(**{'unroll':8})
```

```python
import jax
import jax.numpy as jnp
from jax import lax
import jax.experimental.pallas as pl
import jax.experimental.pallas.tpu as pltpu

B, SQ, D, H, SK, DH = 8, 224, 448, 16, 512, 256
R = B * SQ
HQ, HD, HK, HH, HR = SQ // 2, D // 2, SK // 2, DH // 2, R // 2
STEPS = 2 * H
SCALE = DH ** -0.5
EDGE = 384
BF, F32, U32 = jnp.bfloat16, jnp.float32, jnp.uint32
NN = (((1,), (0,)), ((), ()))
NT = (((1,), (1,)), ((), ()))
TN = (((0,), (0,)), ((), ()))


def _dot(a, b, dims):
    return lax.dot_general(a, b, dims, preferred_element_type=F32)


def _f32(x):
    return x.astype(F32)


def _bf(x):
    return x.astype(BF)


def _to_words(x):
    return pltpu.bitcast(_bf(x), U32)


def _from_words(x):
    return pltpu.bitcast(x, BF)


def _enc_a(x11, x12, x21, x22):
    return [x11 + x22, x21 + x22, x11, x22, x11 + x12, x21 - x11, x12 - x22]


def _enc_b(x11, x12, x21, x22):
    return [x11 + x22, x11, x12 - x22, x21 - x11, x22, x11 + x12, x21 + x22]


_B_UNMIXED = {1: 0, 4: 3}


def _enc_g(x11, x12, x21, x22):
    return [x11 + x22, x21 - x22, x12 + x22, x11 + x21, x12 - x11, x22, x11]


def _sum(m, terms, order):
    terms = sorted(terms, key=lambda term: order.index(term[1]))
    if terms[0][0] < 0:
        terms[0], terms[1] = terms[1], terms[0]
    acc = m[terms[0][1]]
    for sign, i in terms[1:]:
        acc = acc + m[i] if sign > 0 else acc - m[i]
    return acc


_DEC_C = (((1, 0), (1, 3), (-1, 4), (1, 6)), ((1, 2), (1, 4)), ((1, 1), (1, 3)), ((1, 0), (-1, 1), (1, 2), (1, 5)))
_DEC_DA = (((1, 0), (1, 2), (1, 4), (-1, 5)), ((1, 4), (1, 6)), ((1, 1), (1, 5)), ((1, 0), (1, 1), (1, 3), (-1, 6)))
_DEC_DB = (((1, 0), (1, 1), (-1, 3), (1, 5)), ((1, 2), (1, 5)), ((1, 3), (1, 6)), ((1, 0), (-1, 2), (1, 4), (1, 6)))


_SPARE = {"A": {6: (0, 1), 5: (0, 1), 3: (1, 1), 1: (1, -1), 2: (2, 1), 4: (2, -1)},
          "G": {2: (0, 1), 3: (0, 1), 1: (1, 1), 5: (1, -1), 4: (2, 1), 6: (2, -1)}}
_IDLE = 256 - HD


def _fill_idle(name, ys, i, axis):
    if i == 0:
        return jnp.concatenate([ys[0], jnp.zeros_like(lax.slice_in_dim(ys[0], 0, _IDLE, axis=axis))], axis=axis)
    third, sign = _SPARE[name][i]
    piece = lax.slice_in_dim(ys[0], 128 + third * _IDLE, 128 + (third + 1) * _IDLE, axis=axis)
    return jnp.concatenate([ys[i], -piece if sign < 0 and axis == 0 else piece], axis=axis)


def _block_product(dec, order, product):
    m = {i: product(i) for i in order}
    return [_sum(m, terms, order) for terms in dec]


def _quad(x):
    r, c = x.shape[0] // 2, x.shape[1] // 2
    return [x[:r, :c], x[:r, c:], x[r:, :c], x[r:, c:]]


def _chunks(sizes):
    lo = 0
    for n in sizes:
        yield slice(lo, lo + n)
        lo += n


def _shift(sl, off):
    return slice(sl.start + off, sl.stop + off)


def _stack_rows(parts):
    return [jnp.concatenate(p, axis=0) if len(p) > 1 else p[0] for p in zip(*parts)]


def _start(copies):
    for c in copies:
        c.start()


def _wait(copies):
    for c in copies:
        c.wait()


_SEQUENCE = "GAAqssppkkkkkvoGvvvvvvv"
_EDGE_SEQUENCE = {1: "GAAqssppGkkkkkvovvvvvvv", 7: "GAAqossppkkkkkvvvvvvvvG"}
_AHEAD = {"A": 2, "G": 2, "s": 1, "p": 1, "o": 0, "q": 0, "v": 0, "k": 0}
_HEAD_SEQUENCE = "XUFW"
_ROW_CHUNKS = {"A": (48, 64), "G": (48, 64), "o": (112,), "q": (112,),
               "k": (64, 48, 48, 48, 48), "v": (32, 32, 32, 32, 32, 32, 32, 32)}
_PRODUCT_ORDER = {name: [int(c) for c in order] for name, order in {
    "A": "1534602", "G": "4516230", "s": "4320165", "p": "4612053", "o": "1024635",
    "q": "4615023", "v": "0532641", "k": "3065142", "W": "2534106", "U": "2365014"}.items()}


def _kernel(xa, ka, va, wqa, woa, xb, kb, vb, wqb, wob, g_hbm,
            out_hbm, dxa, dka, dva, dwqa, dwoa, dxb, dkb, dvb, dwqb, dwob,
            x_s, g_s, ax_s, gg_s, k_s, v_s, wq_s, wo_s, dk_s, dv_s, dwq_s, dwo_s,
            bw_s, ao_s, gdq_s, out_acc, dx_acc, edge_s, out_s, dx_s, isem, osem, msem, rsem):
    def kv_copies(branch, h, slot):
        return [pltpu.make_async_copy((ka, kb)[branch].at[:, h], k_s.at[slot], isem.at[0, slot]),
                pltpu.make_async_copy((va, vb)[branch].at[:, h], v_s.at[slot], isem.at[1, slot])]

    def dkv_copies(branch, h, slot):
        return [pltpu.make_async_copy(dk_s.at[slot], (dka, dkb)[branch].at[:, h], osem.at[0, slot]),
                pltpu.make_async_copy(dv_s.at[slot], (dva, dvb)[branch].at[:, h], osem.at[1, slot])]

    def w_copies(branch, lo, hi, sem):
        col = slice(lo * DH, hi * DH)
        return [pltpu.make_async_copy((wqa, wqb)[branch].at[:, col], wq_s.at[branch, :, col], msem.at[sem]),
                pltpu.make_async_copy((woa, wob)[branch].at[:, col], wo_s.at[branch, :, col], msem.at[sem + 1])]

    def dw_copies(branch, lo, hi, sem):
        col = slice(lo * DH, hi * DH)
        return [pltpu.make_async_copy(dwq_s.at[branch, :, col], (dwqa, dwqb)[branch].at[:, col], msem.at[sem]),
                pltpu.make_async_copy(dwo_s.at[branch, :, col], (dwoa, dwob)[branch].at[:, col], msem.at[sem + 1])]

    def xg_copies(branch):
        col = slice(branch * EDGE, branch * EDGE + 512)
        return [pltpu.make_async_copy((xa, xb)[branch], x_s.at[branch], msem.at[0]),
                pltpu.make_async_copy(g_hbm.at[:, col], g_s.at[branch], msem.at[1])]

    def result_copy(name, branch, r):
        if name == "dx":
            return pltpu.make_async_copy(dx_s.at[branch, :, r], (dxa, dxb)[branch].at[:, r], rsem.at[branch, r])
        col = slice(EDGE, 2 * D) if branch else slice(0, EDGE)
        return pltpu.make_async_copy(out_s.at[branch, :, r, :, :col.stop - col.start], out_hbm.at[:, r, :, col],
                                     rsem.at[branch, 2 + r])

    def for_step(t, fn):
        pl.when(t < H)(lambda: fn(0, t))
        pl.when(jnp.logical_and(t >= H, t < STEPS))(lambda: fn(1, t - H))

    def head_cols(t):
        return pl.ds(pl.multiple_of((t % H) * DH, DH), DH)

    def encode_rows(name, src, col, slot, b):
        enc, dst = (_enc_a, ax_s) if name == "A" else (_enc_g, gg_s)
        top = _f32(src[pl.ds(pl.multiple_of(b * SQ, 16), HQ), col:col + D])
        bot = _f32(src[pl.ds(pl.multiple_of(b * SQ + HQ, 16), HQ), col:col + D])
        rows = pl.ds(pl.multiple_of(b * (HQ // 2), 8), HQ // 2)
        ys = enc(top[:, :HD], top[:, HD:], bot[:, :HD], bot[:, HD:])
        for i in range(7):
            dst[slot, i, rows, :] = _to_words(_fill_idle(name, ys, i, 1))

    def encode_weights(branch, col):
        yq = _enc_b(*_quad(_f32(wq_s[branch, :, col]) * SCALE))
        t11, t12, t21, t22 = _quad(_f32(wo_s[branch, :, col]))
        yo = _enc_b(t11, t21, t12, t22)
        for i in range(7):
            bw_s[i] = _to_words(jnp.concatenate([_fill_idle("A", yq, i, 0), _fill_idle("G", yo, i, 0)], axis=1))

    def project(u, branch, st, name):
        src, col, dec, enc = ((ax_s, slice(0, HH), _DEC_C, _enc_a) if name == "A" else
                              (gg_s, slice(HH, DH), _DEC_DA, _enc_g))
        parts = []
        for ch in _chunks(_ROW_CHUNKS[name]):
            rows = slice((u * HQ + ch.start) // 2, (u * HQ + ch.stop) // 2)
            parts.append(_block_product(dec, _PRODUCT_ORDER[name], lambda i: _dot(
                _from_words(src[branch, i, rows, :256 if i else 128]),
                _from_words(bw_s[i, :128 if i else 64, col]), NN)))
            if ch.stop == HQ:
                st[name] = [_bf(y) for y in enc(*_stack_rows(parts))]
            yield

    def cache_operand(raw, blocks, u, slot, zero):
        mixed = [_enc_b(*[_f32(raw[slot + zero * (i + 1), u, r, c]) for r, c in blocks])[i] for i in range(7)]

        def get(i, keys):
            if i in _B_UNMIXED:
                r, c = blocks[_B_UNMIXED[i]]
                return raw[slot, u, _shift(keys, r.start), c]
            return _bf(mixed[i][keys])
        return get

    def scores(st, name):
        lhs, rhs, dec = ("A", "K", _DEC_C) if name == "s" else ("G", "V", _DEC_DA)
        cols = []
        for keys in _chunks((128, 128)):
            cols.append(_block_product(dec, _PRODUCT_ORDER[name], lambda i: _dot(st[lhs][i], st[rhs](i, keys), NT)))
            if keys.stop == HK:
                c11, c12, c21, c22 = [list(p) for p in zip(*cols)]
                st[name] = (jnp.concatenate(c11 + c12, axis=1), jnp.concatenate(c21 + c22, axis=1))
            yield

    def softmax(st, name):
        if "P" not in st:
            ps, ds = [], []
            for s, dp in zip(st["s"], st["p"]):
                e = jnp.exp(s - jnp.max(s, axis=1, keepdims=True))
                p = e * (1.0 / jnp.sum(e, axis=1, keepdims=True))
                ps.append(p)
                ds.append(p * (dp - jnp.sum(p * dp, axis=1, keepdims=True)))
            st["P"] = _enc_a(ps[0][:, :HK], ps[0][:, HK:], ps[1][:, :HK], ps[1][:, HK:])
            st["dS"] = _enc_g(ds[0][:, :HK], ds[0][:, HK:], ds[1][:, :HK], ds[1][:, HK:])
        return st[name]

    def row_product(u, st, name):
        lhs, rhs, dec, enc, dst = (("P", "V", _DEC_C, _enc_a, ao_s) if name == "o" else
                                   ("dS", "K", _DEC_DA, _enc_g, gdq_s))
        ys = softmax(st, lhs)
        for ch in _chunks(_ROW_CHUNKS[name]):
            z = enc(*_block_product(dec, _PRODUCT_ORDER[name], lambda i: _dot(
                _bf(ys[i][ch]), st[rhs](i, slice(0, HK)), NN)))
            rows = slice((u * HQ + ch.start) // 2, (u * HQ + ch.stop) // 2)
            for j in range(4):
                dst[j, rows, :] = _to_words(jnp.concatenate([z[2 * j], z[min(2 * j + 1, 6)]], axis=1))
            yield

    def key_product(u, slot, st, name):
        lhs, rhs, dst = ("P", "G", dv_s) if name == "v" else ("dS", "A", dk_s)
        lt = [_bf(y).T for y in softmax(st, lhs)]
        for ch in _chunks(_ROW_CHUNKS[name]):
            d11, d12, d21, d22 = _block_product(_DEC_DB, _PRODUCT_ORDER[name], lambda i: _dot(lt[i][ch], st[rhs][i], NN))
            if name == "k":
                d12, d21 = d21, d12
            dst[slot, u, ch, :] = _bf(jnp.concatenate([d11, d12], axis=1))
            dst[slot, u, _shift(ch, HK), :] = _bf(jnp.concatenate([d21, d22], axis=1))
            yield

    def batch_tasks(u, branch, slot, zero):
        lo, hi, left, right = slice(0, HK), slice(HK, SK), slice(0, HH), slice(HH, DH)
        st = {"K": cache_operand(k_s, [(lo, left), (hi, left), (lo, right), (hi, right)], u, slot, zero),
              "V": cache_operand(v_s, [(lo, left), (lo, right), (hi, left), (hi, right)], u, slot, zero)}
        return {"A": project(u, branch, st, "A"), "G": project(u, branch, st, "G"),
                "s": scores(st, "s"), "p": scores(st, "p"),
                "o": row_product(u, st, "o"), "q": row_product(u, st, "q"),
                "v": key_product(u, slot, st, "v"), "k": key_product(u, slot, st, "k")}

    def stored(ref, i):
        return _from_words(ref[i // 2, :, (i % 2) * HH:(i % 2 + 1) * HH])

    def accumulate(t, name):
        acc, col, y = (out_acc, slice(HH, DH), ao_s) if name == "F" else (dx_acc, slice(0, HH), gdq_s)
        for i in range(7):
            m = _dot(_from_words(bw_s[i, :HD // 2, col]), stored(y, i), NT)
            acc[i] = jnp.where(t % H == 0, 0.0, acc[i]) + m

    def weight_grad(t, name):
        src, rhs, dst = (gg_s, ao_s, dwo_s) if name == "U" else (ax_s, gdq_s, dwq_s)
        d11, d12, d21, d22 = _block_product(_DEC_DB, _PRODUCT_ORDER[name], lambda i: _dot(
            _from_words(src[t // H, i])[:, :HD], stored(rhs, i), TN))
        if name == "U":
            d12, d21 = d21, d12
        else:
            d11, d12, d21, d22 = d11 * SCALE, d12 * SCALE, d21 * SCALE, d22 * SCALE
        dst[t // H, :HD, head_cols(t)] = _bf(jnp.concatenate([d11, d12], axis=1))
        dst[t // H, HD:, head_cols(t)] = _bf(jnp.concatenate([d21, d22], axis=1))

    def finalize(name, branch):
        acc, dec, dst = (out_acc, _DEC_C, out_s) if name == "out" else (dx_acc, _DEC_DA, dx_s)
        c11, c12, c21, c22 = _block_product(dec, list(range(7)), lambda i: acc[i])
        for r, (lo, hi) in enumerate(((c11, c12), (c21, c22))):
            if name == "dx":
                y = jnp.concatenate([lo, hi], axis=0)
            elif branch == 0:
                y = jnp.concatenate([lo, hi[:EDGE - HD]], axis=0)
                edge_s[r] = hi[EDGE - HD:]
            else:
                y = jnp.concatenate([edge_s[r], lo, hi], axis=0)
            y = _bf(y).T
            for b in range(B):
                dst[branch, b, r, :, :y.shape[1]] = y[b * HQ:(b + 1) * HQ]
            if branch == 1:
                result_copy(name, branch, r).start()

    first_xg, first_w = xg_copies(0), w_copies(0, 0, 1, 2)
    _start(first_xg + first_w + kv_copies(0, 0, 0))
    first_xg[0].wait()
    lax.fori_loop(0, B, lambda b, c: encode_rows("A", x_s.at[0], 0, 0, b), None)
    first_xg[1].wait()
    lax.fori_loop(0, B, lambda b, c: encode_rows("G", g_s.at[0], 0, 0, b), None)
    _wait(first_w)
    encode_weights(0, slice(0, DH))
    _wait(kv_copies(0, 0, 0))
    _start(kv_copies(0, 1, 1) + w_copies(0, 1, H, 2))

    def step(t, carry):
        slot, branch, zero = t % 2, t // H, t >> 16

        tasks = [batch_tasks(u, branch, slot, zero) for u in range(B)]
        for n in range(-max(_AHEAD.values()), B - min(_AHEAD.values())):
            for name in _EDGE_SEQUENCE.get(n, _SEQUENCE):
                if 0 <= n + _AHEAD[name] < B:
                    next(tasks[n + _AHEAD[name]][name])

        for_step(t, lambda br, h: _start(dkv_copies(br, h, slot)))
        for_step(t + 2, lambda br, h: _start(kv_copies(br, h, slot)))
        for buf, col in ((dk_s, slice(0, HH)), (dv_s, slice(HH, DH))):
            buf[2 + zero, 0, :16, :HH] = _from_words(bw_s[6, :8, col])
            bw_s[6, :8, col] = pltpu.bitcast(buf[2 + (t >> 17), 0, :16, :HH], U32)
        for name in _HEAD_SEQUENCE:
            (accumulate if name in "FX" else weight_grad)(t, name)

        nxt = jnp.where(t == 0, 0, jnp.minimum(t + 1, STEPS - 1))
        encode_weights(nxt // H, head_cols(nxt))
        src = jnp.minimum(t // 2, 1)
        encode_rows("A", x_s.at[src], 0, 1 - branch, t % B)
        encode_rows("G", g_s.at[src], D - EDGE, 1 - branch, t % B)

        pl.when(t + 1 < STEPS)(lambda: _wait(kv_copies(0, 0, 1 - slot)))
        pl.when(t >= 1)(lambda: _wait(dkv_copies(0, 0, 1 - slot)))

        @pl.when(jnp.logical_or(t < 3, t % H >= H - 2))
        def _():
            @pl.when(t == 0)
            def _():
                _wait(w_copies(0, 1, H, 2))
                _start(xg_copies(1))
                encode_weights(0, slice(DH, 2 * DH))

            @pl.when(t == 1)
            def _():
                _wait(xg_copies(1))
                _start(w_copies(1, 0, H, 4))

            pl.when(t == 2)(lambda: _wait(w_copies(1, 0, H, 4)))
            pl.when(t == STEPS - 2)(lambda: _start(dw_copies(1, 0, H - 1, 4)))

            @pl.when(t == H - 1)
            def _():
                finalize("out", 0)
                finalize("dx", 0)
                _start([result_copy(name, 0, r) for name in ("out", "dx") for r in range(2)])
                _start(dw_copies(0, 0, H, 2))
        return carry

    lax.fori_loop(0, STEPS, step, 0)
    _wait(dw_copies(0, 0, H, 2))
    _start(dw_copies(1, H - 1, H, 2))
    finalize("dx", 1)
    finalize("out", 1)
    _wait(dkv_copies(1, H - 1, 1))
    _wait(dw_copies(1, 0, H - 1, 4) + dw_copies(1, H - 1, H, 2))
    _wait([result_copy(name, br, r) for name in ("dx", "out") for br in range(2) for r in range(2)])


@jax.jit
def pallas_concat_heads__mha_block_cached__gqa_block_cached__near_ridge_kernel(
        A_x, A_k_cache, A_v_cache, A_wq, A_wo, B_x, B_k_cache, B_v_cache, B_wq, B_wo, grad_out):
    sds, vmem = jax.ShapeDtypeStruct, pltpu.VMEM
    grads = [sds((B, 2, HQ, D), BF), sds((B, H, SK, DH), BF), sds((B, H, SK, DH), BF),
             sds((D, H * DH), BF), sds((D, H * DH), BF)]
    rows, cache, dcache = vmem((2, 7, HR // 2, 256), U32), vmem((2, B, SK, DH), BF), vmem((3, B, SK, DH), BF)
    weight, head, acc = vmem((2, D, H * DH), BF), vmem((4, HR // 2, DH), U32), vmem((7, HD, HR), F32)
    in_hbm = pl.BlockSpec(memory_space=pl.ANY)
    out, dxa, dka, dva, dwqa, dwoa, dxb, dkb, dvb, dwqb, dwob = pl.pallas_call(
        _kernel,
        out_shape=[sds((B, 2, HQ, 2 * D), BF)] + grads + grads,
        in_specs=[in_hbm] * 11,
        out_specs=[in_hbm] * 11,
        scratch_shapes=[
            vmem((2, R, D), BF), vmem((2, R, 512), BF), rows, rows, cache, cache, weight, weight,
            dcache, dcache, weight, weight, vmem((7, 128, DH), U32), head, head, acc, acc,
            vmem((2, D - EDGE, HR), F32), vmem((2, B, 2, HQ, 512), BF), vmem((2, B, 2, HQ, D), BF),
            pltpu.SemaphoreType.DMA((2, 2)), pltpu.SemaphoreType.DMA((2, 2)),
            pltpu.SemaphoreType.DMA((6,)), pltpu.SemaphoreType.DMA((2, 4)),
        ],
        compiler_params=pltpu.CompilerParams(
            vmem_limit_bytes=120 * 2 ** 20, disable_bounds_checks=True,
            flags={"XLA_TPU_EVENLY_DISTRIBUTE_CRITICAL_NODES": True}),
    )(A_x.reshape(R, D), A_k_cache, A_v_cache, A_wq, A_wo.T,
      B_x.reshape(R, D), B_k_cache, B_v_cache, B_wq, B_wo.T, grad_out.reshape(R, 2 * D))
    return (out.reshape(B, SQ, 2 * D), dxa.reshape(B, SQ, D), dka, dva, dwqa, dwoa.T,
            dxb.reshape(B, SQ, D), dkb, dvb, dwqb, dwob.T)
```
